```python
import jax
import jax.numpy as jnp

def _softmax(x, axis=-1):
    return jax.nn.softmax(x, axis=axis)
def _gelu(x):
    return jax.nn.gelu(x, approximate=True)
def _silu(x):
    return jax.nn.silu(x)
def _sigmoid(x):
    return jax.nn.sigmoid(x)
def _layernorm(x, axis=-1, eps=1e-5):
    m = jnp.mean(x, axis=axis, keepdims=True)
    v = jnp.var(x, axis=axis, keepdims=True)
    return (x - m) / jnp.sqrt(v + eps)
def _scatter_add(tgt, idx, src, axis=0):
    return tgt.at[idx].add(src)
def _segment_sum(src, seg, n):
    return jax.ops.segment_sum(src, seg, n)
class _Rng:
    def __init__(self, key):
        self._k = key
    def _next(self):
        self._k, sub = jax.random.split(self._k)
        return sub
    def normal(self, shape):
        return jax.random.normal(self._next(), shape, dtype=jnp.bfloat16)
    def randint(self, lo, hi, shape):
        return jax.random.randint(self._next(), shape, lo, hi, dtype=jnp.int32)
    def uniform(self, shape, lo=0.0, hi=1.0):
        return jax.random.uniform(self._next(), shape, jnp.bfloat16, lo, hi)
    def permutation(self, n):
        return jax.random.permutation(self._next(), n)


kernel_name = 'gated_mix__sliding_local_dilated__swiglu_ffn__prompt'

def _fwd_setup_inputs():
    _rng = _Rng(jax.random.key(int.from_bytes(__import__("os").urandom(4), "little")))
    _w = (lambda a: (lambda t: t.astype(jnp.bfloat16) if jnp.issubdtype(t.dtype, jnp.floating) else t)(jnp.asarray(a)))
    def _A_setup():
        B, S, D = 1, 2048, 448
        return {
            "x": _w((lambda *s: _rng.normal(s) * 0.05)(B, S, D)),
            "wqkv": _w((lambda *s: _rng.normal(s) * 0.05)(D, 3 * D)),
            "wo": _w((lambda *s: _rng.normal(s) * 0.05)(D, D)),
        }
    _A_in = _A_setup()

    def _B_setup():
        B, S, D, F = 1, 2048, 448, 1792
        return {
            "x": _w((lambda *s: _rng.normal(s) * 0.05)(B, S, D)),
            "w_gate": _w((lambda *s: _rng.normal(s) * 0.05)(D, F)),
            "w_up": _w((lambda *s: _rng.normal(s) * 0.05)(D, F)),
            "w_down": _w((lambda *s: _rng.normal(s) * 0.05)(F, D)),
        }
    _B_in = _B_setup()

    return {
        "A_x": _A_in["x"],
        "A_wqkv": _A_in["wqkv"],
        "A_wo": _A_in["wo"],
        "B_x": _B_in["x"],
        "B_w_gate": _B_in["w_gate"],
        "B_w_up": _B_in["w_up"],
        "B_w_down": _B_in["w_down"],
        "gate_w": _w((lambda *s: _rng.normal(s) * 0.05)(448)),
    }

def _fwd_reference(A_x, A_wqkv, A_wo, B_x, B_w_gate, B_w_up, B_w_down, gate_w):
    def _A_ref(x, wqkv, wo):
        B, S, D = x.shape
        H = 16; Dh = D // H
        W, dil = 8, 2
        qkv = (lambda x, *d: x.transpose(*d))((x @ wqkv).reshape(B, S, 3, H, Dh), 2, 0, 3, 1, 4)
        q, k, v = qkv[0], qkv[1], qkv[2]
        scale = Dh ** -0.5
        pos = jnp.arange(S)
        off = jnp.arange(W) * dil
        idx = pos[:, None] - off[None, :]
        mask = idx >= 0
        idx_c = jnp.where(mask, idx, 0).reshape(-1)
        kg = k[:, :, idx_c, :].reshape(B, H, S, W, Dh)
        vg = v[:, :, idx_c, :].reshape(B, H, S, W, Dh)
        logits = jnp.einsum("bhsd,bhswd->bhsw", q, kg) * scale
        logits = jnp.where(mask[None, None, :, :], logits, -1e9)
        attn = _softmax(logits, axis=-1)
        o = jnp.einsum("bhsw,bhswd->bhsd", attn, vg)
        return (lambda x, *d: x.transpose(*d))(o, 0, 2, 1, 3).reshape(B, S, D) @ wo

    def _B_ref(x, w_gate, w_up, w_down):
        g = _silu(x @ w_gate)
        u = x @ w_up
        return (g * u) @ w_down

    x = A_x
    g = _sigmoid((x * gate_w).sum(-1, keepdims=True))
    a = _A_ref(x, A_wqkv, A_wo)
    b = _B_ref(x, B_w_gate, B_w_up, B_w_down)
    return g * a + (1 - g) * b


def setup_inputs():
    _inp = _fwd_setup_inputs()
    _gk = jax.random.fold_in(jax.random.key(int.from_bytes(__import__("os").urandom(4), "little")), 2**31 - 1)
    _shapes = [[1, 2048, 448]]
    _dtypes = ['bfloat16']
    _gks = jax.random.split(_gk, len(_shapes))
    _gs = [jax.random.normal(k, s, dtype=jnp.dtype(d)) * 0.05 for k, s, d in zip(_gks, _shapes, _dtypes)]
    _inp["grad_out"] = _gs[0]
    return _inp

def reference(A_x, A_wqkv, A_wo, B_w_gate, B_w_up, B_w_down, gate_w, B_x, grad_out):
    _const = dict(B_x=B_x)
    def _f(*_d):
        return _fwd_reference(**{'A_x': _d[0], 'A_wqkv': _d[1], 'A_wo': _d[2], 'B_w_gate': _d[3], 'B_w_up': _d[4], 'B_w_down': _d[5], 'gate_w': _d[6], **_const})
    _out, _vjp = jax.vjp(_f, A_x, A_wqkv, A_wo, B_w_gate, B_w_up, B_w_down, gate_w)
    _grads = _vjp(grad_out)
    _out0 = jnp.asarray(_out)
    return (_out0, *[jnp.asarray(_g) for _g in _grads])
```

```python
import functools

import jax
import jax.numpy as jnp
from jax import lax
from jax.experimental import pallas as pl
from jax.experimental.pallas import tpu as pltpu

S = 2048
D = 448
DP = 512
H = 16
DH = 28
W = 8
F = 1792
NF = F // 128
NL = S // 128
NT = NL // 2
QKV = 3 * D
NQ = 11
QKVP = NQ * 128
SCALE = float(DH) ** -0.5

f32 = jnp.float32
bf16 = jnp.bfloat16
u32 = jnp.uint32

NH = 8
D_STEPS = 4
E_ROWS = 16
ATT_END = 0.95
DY_CUTS = (0, 1, 3, 6, 11, NL)
W_CUTS = (0, 1, 3, 6, NF)
X_CUTS = (0, 2, NL)

NSEM_IN = 24
SEM_OUT, SEM_DX, SEM_DWG, SEM_DWU, SEM_DWD, SEM_DWO, SEM_DWQ, SEM_DGW = (
    NSEM_IN + i for i in range(8))
NSEM = NSEM_IN + 8

_nn = functools.partial(jnp.dot, preferred_element_type=f32)
_nt = functools.partial(lax.dot_general,
                        dimension_numbers=(((1,), (1,)), ((), ())),
                        preferred_element_type=f32)


def _cat(parts):
    return jnp.concatenate(parts, axis=1)


def _ld(ref, idx, r0, r1):
    return pltpu.bitcast(ref[idx + (pl.ds(r0 // 2, (r1 - r0) // 2),)], bf16)


def _st(ref, idx, r0, val):
    ref[idx + (pl.ds(r0 // 2, val.shape[0] // 2),)] = pltpu.bitcast(val, u32)


class Unit:
    def __init__(self, cost, fn, needs=(), gives=(), steps=0, groups=1):
        self.cost, self.fn = cost, fn
        self.steps = steps
        self.groups = groups
        self.needs, self.gives = set(needs), set(gives)


class Queue:
    def __init__(self, units, t0, t1, per_chunk=1 << 30):
        self.units, self.t0, self.t1 = list(units), t0, t1
        self.per_chunk = per_chunk
        self.total = sum(u.cost for u in self.units)
        self.spent = 0
        self.pos = 0

    def target(self, t):
        if self.t1 <= self.t0:
            return self.total if t >= self.t0 else 0
        frac = (t - self.t0) / (self.t1 - self.t0)
        return self.total * min(max(frac, 0.0), 1.0)


def emit(chunks, queues, lazy):
    done = set()
    last = [None, 1]
    rel = {}
    state = dict(j=0, m=1)
    provider = {g: u for u in lazy for g in u.gives}
    where = {g: (q, i) for q in queues for i, u in enumerate(q.units)
             for g in u.gives}

    def release():
        res, groups = last
        j, m = min(state["j"], state["m"] - 1), state["m"]
        state["j"] += 1
        rows = res.shape[0] // 8
        per = res.shape[1] // 128 // groups
        pos = rows * groups * j // m
        r, c = (pos % rows) * 8, (pos // rows) * per * 128
        if (r, c) not in rel:
            rel[(r, c)] = jnp.minimum(jnp.abs(res[r:r + 8, c:c + 128]), 0.0)
        return rel[(r, c)]

    def run(u):
        for n in sorted(u.needs - done, key=str):
            force(n)
        if u.steps:
            u.fn(release)
        else:
            u.fn()
        done.update(u.gives)

    def step_queue(q):
        u = q.units[q.pos]
        q.pos += 1
        q.spent += u.cost
        run(u)

    def force(tok):
        if tok in done:
            return
        if tok in provider:
            run(provider[tok])
            return
        q, i = where[tok]
        while q.pos <= i:
            step_queue(q)

    def ready(u, extra):
        return all(n in done or n in extra
                   or (n in provider and ready(provider[n], extra))
                   for n in u.needs)

    t = 0
    for c in chunks:
        for n in sorted(c.needs - done, key=str):
            force(n)
        res = c.fn()
        if c.cost > 0:
            last[:] = [res, c.groups]
            rel.clear()
        done.update(c.gives)
        t += c.cost
        batch = []
        for q in queues:
            pos, spent, extra, n = q.pos, q.spent, set(), 0
            while (pos < len(q.units) and spent < q.target(t)
                   and n < q.per_chunk and ready(q.units[pos], extra)):
                u = q.units[pos]
                batch.append((q, u))
                extra |= u.gives
                spent += u.cost
                pos += 1
                n += 1
        state["j"] = 0
        state["m"] = max(sum(u.steps for _, u in batch), 1)
        for q, u in batch:
            if q.pos < len(q.units) and q.units[q.pos] is u:
                step_queue(q)
    assert all(q.pos == len(q.units) for q in queues)


def _kernel(xT_h, wq_h, wo_h, wg_h, wu_h, wd_h, gw_h, dyT_h,
            out_h, dx_h, dwq_h, dwo_h, dwg_h, dwu_h, dwd_h, dgw_h,
            wq_raw, wo_raw, gw_raw, x_raw, dy_raw, wg_raw, wu_raw, wd_raw,
            gwb, xT, dyT, wgu, wd, wguL, wdL, wqkv, wqkvT, wo, woT,
            qkv, pp, gs, lg, da, pr, at, dl, dga,
            o_st, dq_st, dk_st, dv_st, oT, dqkv,
            xb, dy, xbTs, dbT, gu_s, q_s, h_s, dgu_s,
            bT, gaT, xfT, awg, awu, awd, awo, awq,
            out_st, dx_st, dwg_st, dwu_st, dwd_st, dwo_st,
            dwq_st, dwq_se, dgw_st,
            sem):

    def cp(src, dst, s):
        return pltpu.make_async_copy(src, dst, sem.at[s])

    in_flight = {}
    in_sems = []

    def start_in(name, src, dst, t0=None, t1=None):
        if t0 is not None:
            cols = pl.ds(t0 * 128, (t1 - t0) * 128)
            src, dst = src.at[:, cols], dst.at[:, cols]
        in_sems.append(len(in_sems))
        in_flight[(name, t0)] = (src, dst, in_sems[-1])
        cp(src, dst, in_sems[-1]).start()

    def pieces(key):
        name, t0 = key
        if t0 is None:
            return [name]
        cuts = dict(dy=DY_CUTS, x=X_CUTS).get(name, W_CUTS)
        return [(name, i) for i in range(t0, cuts[cuts.index(t0) + 1])]

    def barrier(keys, then=None):
        def fn():
            for k in keys:
                cp(*in_flight.pop(k)).wait()
            if then is not None:
                then()
        return Unit(0, fn, gives=[("dma", g) for k in keys for g in pieces(k)])

    out_flight = []

    def start_out(src, dst, s):
        out_flight.append((src, dst, s))
        cp(src, dst, s).start()

    def start_w(i):
        for nm, h_, r_ in (("wg", wg_h, wg_raw), ("wu", wu_h, wu_raw),
                           ("wd", wd_h, wd_raw)):
            start_in(nm, h_, r_, W_CUTS[i], W_CUTS[i + 1])

    def w_keys(i):
        return [(nm, W_CUTS[i]) for nm in ("wg", "wu", "wd")]

    dy_groups = list(zip(DY_CUTS[:-1], DY_CUTS[1:]))
    start_in("wo", wo_h, wo_raw)
    for a, b in dy_groups[:2]:
        start_in("dy", dyT_h, dy_raw, a, b)

    def start_rest():
        for a, b in dy_groups[2:]:
            start_in("dy", dyT_h, dy_raw, a, b)
        start_in("x", xT_h, x_raw, X_CUTS[0], X_CUTS[1])
        start_in("gw", gw_h, gw_raw)
        start_w(0)
        start_w(1)
        start_in("wq", wq_h, wq_raw)
        start_w(2)
        start_w(3)
        start_in("x", xT_h, x_raw, X_CUTS[1], X_CUTS[2])

    lane16 = lax.broadcasted_iota(jnp.int32, (H, 128), 1)
    lane8 = lax.broadcasted_iota(jnp.int32, (NH, 128), 1)

    def zeros(shape, dt):
        return jnp.zeros(shape, dt)

    def col(raw, i):
        return raw[:, i * 128:(i + 1) * 128]

    lazy = []

    def padded(tile):
        return jnp.concatenate([tile, zeros((DP - D, 128), bf16)], axis=0)

    def repack_unit(name, raw, i, dst):
        def fn():
            dst[i] = pltpu.bitcast(padded(col(raw, i)), u32)
        lazy.append(Unit(30, fn, needs=[("dma", (name, i))],
                         gives=[(name + "T", i)]))

    for L in range(NL):
        repack_unit("dy", dy_raw, L, dyT)
        repack_unit("x", x_raw, L, xT)

    def w_units(f):
        needs = [("dma", (n, f)) for n in ("wg", "wu", "wd")]

        def as_rhs():
            g, u, d_ = col(wg_raw, f), col(wu_raw, f), col(wd_raw, f)
            wgu[f, 0] = pltpu.bitcast(padded(g), u32)
            wgu[f, 1] = pltpu.bitcast(padded(u), u32)
            wd[f] = pltpu.bitcast(padded(d_), u32)
        lazy.append(Unit(60, as_rhs, needs=needs, gives=[("w", f)]))

        def as_lhs():
            wguL[f, 0] = pltpu.bitcast(col(wg_raw, f), u32)
            wguL[f, 1] = pltpu.bitcast(col(wu_raw, f), u32)
            wdL[f] = pltpu.bitcast(col(wd_raw, f), u32)
        lazy.append(Unit(60, as_lhs, needs=needs, gives=[("wL", f)]))

    for f in range(NF):
        w_units(f)

    def end_tile(raw, c0):
        return _cat([raw[:, c0:c0 + 64], zeros((D, 64), bf16)])

    def prep_wo():
        for k in range(3):
            wo[k] = pltpu.bitcast(col(wo_raw, k), u32)
        wo[3] = pltpu.bitcast(end_tile(wo_raw, 384), u32)
    lazy.append(Unit(60, prep_wo, needs=[("dma", "wo")], gives=["wo"]))

    def wot_unit(kt):
        def fn():
            r0 = kt * 128
            r1 = min(r0 + 128, D)
            blk = _cat([_ld(wo, (k,), r0, r1) for k in range(4)])
            if r1 - r0 < 128:
                blk = jnp.concatenate(
                    [blk, zeros((128 - (r1 - r0), DP), bf16)], axis=0)
            _st(woT, (kt,), 0, blk.T[0:D, :])
        lazy.append(Unit(150, fn, needs=["wo"], gives=[("woT", kt)]))

    for kt in range(4):
        wot_unit(kt)

    def gwb_unit():
        row = gw_raw[...].reshape(1, D).astype(f32)
        gwb[...] = jnp.broadcast_to(row, (128, D)).T
    lazy.append(Unit(150, gwb_unit, needs=[("dma", "gw")], gives=["gwb"]))

    def wq_unit(j):
        def fn():
            if j < NQ - 1:
                tile = col(wq_raw, j)
            else:
                li = lax.broadcasted_iota(jnp.int32, (D, 128), 1)
                tile = jnp.where(li == 64, gwb[...],
                                 end_tile(wq_raw, 1280).astype(f32)).astype(bf16)
            wqkv[j] = pltpu.bitcast(tile, u32)
            tile = padded(tile)
            for kt in range(4):
                _st(wqkvT, (kt,), j * 128, tile[kt * 128:(kt + 1) * 128, :].T)
        needs = [("dma", "wq")] + (["gwb"] if j == NQ - 1 else [])
        return Unit(250, fn, needs=needs, gives=[("wq", j)])

    wq_prep = [wq_unit(j) for j in range(NQ)]

    def gate_unit(L):
        def fn():
            z = jnp.sum(col(x_raw, L).astype(f32) * gwb[...], axis=0,
                        keepdims=True)
            gs[L] = jnp.broadcast_to(jax.nn.sigmoid(z), (8, 128))
        lazy.append(Unit(60, fn, needs=[("dma", ("x", L)), "gwb"],
                         gives=[("g", L)]))

    def tr_unit(L, src, stag, dst, tag):
        def fn():
            for kt in range(4):
                _st(dst, (L // 2, kt), (L % 2) * 128,
                    _ld(src, (L,), kt * 128, (kt + 1) * 128).T)
        lazy.append(Unit(220, fn, needs=[(stag, L)], gives=[(tag, L)]))

    def scale_unit(L, raw, key, dst, tag):
        def fn():
            om = 1.0 - gs[L, 0:1, :]
            _st(dst, (L,), 0, (col(raw, L).astype(f32) * om).astype(bf16))
        lazy.append(Unit(60, fn, needs=[("dma", (key, L)), ("g", L)],
                         gives=[(tag, L)]))

    for L in range(NL):
        gate_unit(L)
        tr_unit(L, dyT, "dyT", dy, "dy")
        tr_unit(L, xT, "xT", xb, "xb")
        scale_unit(L, dy_raw, "dy", dbT, "dbT")
        scale_unit(L, x_raw, "x", xbTs, "xbTs")

    def zero_unit(tag, ref, idx, shape, dt):
        def fn():
            ref[idx] = zeros(shape, dt)
        lazy.append(Unit(10, fn, gives=[tag]))

    zero_unit("kv_halo", qkv, (0, pl.ds(D, 2 * D)), (2 * D, 128), f32)
    zero_unit("q_halo", qkv, (NL + 1, pl.ds(0, D)), (D, 128), f32)
    zero_unit("p_halo", pp, (NL + 1, pl.ds(0, D)), (D, 128), f32)
    zero_unit("at_halo", at, (NL + 1,), (W, H, 128), f32)
    zero_unit("dl_halo", dl, (NL + 1,), (W, H, 128), f32)
    for L in range(NL):
        zero_unit(("oz", L), oT, (L, pl.ds(D // 2, DP // 2 - D // 2)),
                  (DP // 2 - D // 2, 128), u32)

    def heads(ref, i, off, d, h0):
        return ref[i, pl.ds(off + h0 * DH + d, NH, stride=DH), :]

    from_prev = {w: lane8 >= 128 - 2 * w for w in range(1, W)}
    from_next = {w: lane8 < 2 * w for w in range(1, W)}

    def shift_r(cur, prev, w):
        return pltpu.roll(lax.select(from_prev[w], prev, cur), 2 * w, 1)

    def shift_l(cur, nxt, w):
        return pltpu.roll(lax.select(from_next[w], nxt, cur), 128 - 2 * w, 1)

    def head_groups(build, needs, gives):
        units = []
        for h0 in range(0, H, NH):
            fn_of = build(h0)
            for d0 in range(0, DH, D_STEPS):
                d1 = min(d0 + D_STEPS, DH)
                units.append(Unit((W - 1) * 8 * (d1 - d0) // 3 + 4,
                                  fn_of(d0, d1), steps=d1 - d0))
        units[0].needs |= set(needs)
        units[-1].gives |= set(gives)
        return units

    def logit_units(L):
        li = L + 1

        def build(h0):
            acc = [None] * W

            def make(d0, d1):
                def fn(rel):
                    for d in range(d0, d1):
                        a = heads(qkv, li, 0, d, h0)
                        bc = heads(qkv, li, D, d, h0) + rel()
                        bp = heads(qkv, li - 1, D, d, h0)
                        for w in range(W):
                            t = a * (shift_r(bc, bp, w) if w else bc)
                            acc[w] = t if acc[w] is None else acc[w] + t
                    if d1 == DH:
                        for w in range(W):
                            lg[w, h0:h0 + NH, :] = acc[w]
                return fn
            return make

        needs = [("qkv", L)] + ([("qkv", L - 1)] if L else ["kv_halo"])
        return head_groups(build, needs, [("lg", L)])

    def softmax_unit(L):
        li = L + 1

        def fn():
            g = gs[L, 0:1, :]
            lo = [lg[w] * SCALE for w in range(W)]
            if L == 0:
                lo = [lo[0]] + [jnp.where(lane16 >= 2 * w, lo[w], -1e9)
                                for w in range(1, W)]
            m = lo[0]
            for w in range(1, W):
                m = jnp.maximum(m, lo[w])
            e = [jnp.exp(lo[w] - m) for w in range(W)]
            s = e[0]
            for w in range(1, W):
                s = s + e[w]
            r = 1.0 / s
            for w in range(W):
                p = e[w] * r
                pr[w] = p
                at[li, w] = p * g
        return Unit(40, fn, needs=[("lg", L), ("g", L)], gives=[("p", L)])

    def value_units(L):
        li = L + 1

        def build(h0):
            acc = [None] * W
            coef = [None] * W

            def make(d0, d1):
                def fn(rel):
                    if d0 == 0:
                        for w in range(W):
                            coef[w] = at[li, w, h0:h0 + NH, :]
                    for d in range(d0, d1):
                        a = heads(pp, li, 0, d, h0)
                        bc = heads(qkv, li, 2 * D, d, h0) + rel()
                        bp = heads(qkv, li - 1, 2 * D, d, h0)
                        r = None
                        for w in range(W):
                            bs = shift_r(bc, bp, w) if w else bc
                            t = a * bs
                            acc[w] = t if acc[w] is None else acc[w] + t
                            t = coef[w] * bs
                            r = t if r is None else r + t
                        o_st[pl.ds(h0 * DH + d, NH, stride=DH), :] = r
                    if d1 == DH:
                        for w in range(W):
                            da[w, h0:h0 + NH, :] = acc[w]
                return fn
            return make

        return head_groups(build, [("p", L), ("P", L)], [("v", L)])

    def softmax_bwd_unit(L):
        li = L + 1

        def fn():
            gsc = gs[L, 0:1, :] * SCALE
            p = [pr[w] for w in range(W)]
            dd = [da[w] for w in range(W)]
            dot = p[0] * dd[0]
            for w in range(1, W):
                dot = dot + p[w] * dd[w]
            dga[L] = jnp.broadcast_to(
                jnp.sum(dot, axis=0, keepdims=True), (8, 128))
            for w in range(W):
                dl[li, w] = p[w] * (dd[w] - dot) * gsc
        return Unit(30, fn, needs=[("v", L)], gives=[("dl", L)])

    def combine_units(tag, needs, load_coef, load_pair, shift, dst):
        def build(h0):
            coef = [None] * W

            def make(d0, d1):
                def fn(rel):
                    if d0 == 0:
                        for w in range(W):
                            coef[w] = load_coef(h0, w)
                    for d in range(d0, d1):
                        cur, other = load_pair(d, h0)
                        cur = cur + rel()
                        r = coef[0] * cur
                        for w in range(1, W):
                            r = r + coef[w] * shift(cur, other, w)
                        dst[pl.ds(h0 * DH + d, NH, stride=DH), :] = r
                return fn
            return make

        return head_groups(build, needs, [tag])

    def dq_units(L):
        li = L + 1
        return combine_units(
            ("dqs", L), [("dl", L)],
            lambda h0, w: dl[li, w, h0:h0 + NH, :],
            lambda d, h0: (heads(qkv, li, D, d, h0),
                           heads(qkv, li - 1, D, d, h0)),
            shift_r, dq_st)

    def scatter_units(tag, needs, L, coef_ref, a_ref, dst):
        li = L + 1

        def load_coef(h0, w):
            cur = coef_ref[li, w, h0:h0 + NH, :]
            if w == 0:
                return cur
            return shift_l(cur, coef_ref[li + 1, w, h0:h0 + NH, :], w)
        return combine_units(
            tag, needs, load_coef,
            lambda d, h0: (heads(a_ref, li, 0, d, h0),
                           heads(a_ref, li + 1, 0, d, h0)),
            shift_l, dst)

    def pack_unit(tag, needs, src, dst, L, r0):
        def fn():
            _st(dst, (L,), r0, src[0:D, :].astype(bf16))
        return Unit(20, fn, needs=needs, gives=[tag])

    def fwd_attn(L):
        u = logit_units(L)
        u.append(softmax_unit(L))
        u += value_units(L)
        u.append(pack_unit(("o", L), [("v", L), ("oz", L)], o_st, oT, L, 0))
        u.append(softmax_bwd_unit(L))
        u += dq_units(L)
        u.append(pack_unit(("dq", L), [("dqs", L)], dq_st, dqkv, L, 0))
        return u

    def bwd_attn(L):
        if L + 1 < NL:
            nk = [("dl", L + 1), ("qkv", L + 1)]
            nv = [("dl", L + 1), ("P", L + 1)]
        else:
            nk = ["dl_halo", "q_halo"]
            nv = ["at_halo", "p_halo"]
        u = scatter_units(("dks", L), [("dl", L)] + nk, L, dl, qkv, dk_st)
        u.append(pack_unit(("dk", L), [("dks", L)], dk_st, dqkv, L, D))
        u += scatter_units(("dvs", L), [("dl", L)] + nv, L, at, pp, dv_st)
        u.append(pack_unit(("dv", L), [("dvs", L)], dv_st, dqkv, L, 2 * D))
        return u

    att = fwd_attn(0)
    for L in range(1, NL):
        att += fwd_attn(L)
        att += bwd_attn(L - 1)
    att += bwd_attn(NL - 1)

    def p_chunk(L):
        def fn():
            lhs = _cat([_ld(wo, (k,), 0, D) for k in range(4)])
            res = _nn(lhs, _ld(dyT, (L,), 0, DP))
            pp[L + 1, 0:D, :] = res
            return res
        return Unit(D, fn, needs=["wo", ("dyT", L)], gives=[("P", L)])

    def qkv_chunk(L):
        def fn():
            lhs = _cat([_ld(wqkvT, (kt,), 0, QKV) for kt in range(4)])
            res = _nn(lhs, _ld(xT, (L,), 0, DP))
            qkv[L + 1, 0:QKV, :] = res
            return res
        return Unit(QKV, fn,
                    needs=[("xT", L)] + [("wq", j) for j in range(NQ)],
                    gives=[("qkv", L)])

    def pair(ref, t, r0, r1):
        return _cat([_ld(ref, (2 * t,), r0, r1), _ld(ref, (2 * t + 1,), r0, r1)])

    def nat(ref, t):
        return _cat([_ld(ref, (t, kt), 0, 256) for kt in range(4)])

    def g_chunks(t, f):
        b = f % 2

        def gu():
            rhs = _cat([_ld(wgu, (f, 0), 0, DP), _ld(wgu, (f, 1), 0, DP)])
            res = _nn(nat(xb, t), rhs)
            gu_s[b, 0] = res[:, 0:128]
            gu_s[b, 1] = res[:, 128:256]
            return res

        def q():
            res = _nn(nat(dy, t), _ld(wd, (f,), 0, DP))
            q_s[b] = res
            return res
        return [Unit(512, gu, needs=[("xb", 2 * t), ("xb", 2 * t + 1), ("w", f)],
                     gives=[("gu", t, f)]),
                Unit(256, q, needs=[("dy", 2 * t), ("dy", 2 * t + 1), ("w", f)],
                     gives=[("q", t, f)])]

    def e_units(t, f):
        b = f % 2

        def mk(r0):
            def fn():
                r1 = r0 + E_ROWS
                z = gu_s[b, 0, r0:r1, :]
                u = gu_s[b, 1, r0:r1, :]
                q = q_s[b, r0:r1, :]
                sg = 0.5 * jnp.tanh(0.5 * z) + 0.5
                si = z * sg
                _st(h_s, (b,), r0, (si * u).astype(bf16))
                dsi = sg + si * (1.0 - sg)
                _st(dgu_s, (b, 0), r0, (q * u * dsi).astype(bf16))
                _st(dgu_s, (b, 1), r0, (q * si).astype(bf16))
            return fn
        return [Unit(E_ROWS // 2, mk(r0), needs=[("gu", t, f), ("q", t, f)],
                     gives=[("e", t, f)] if r0 + E_ROWS == 256 else [])
                for r0 in range(0, 256, E_ROWS)]

    def accumulate(t, acc, idx, val, finish):
        v = val if t == 0 else acc[idx] + val
        if t == NT - 1:
            finish(v)
        else:
            acc[idx] = v

    def dw_finish(st, hbm, s, f):
        def finish(v):
            st[:, f * 128:(f + 1) * 128] = v.astype(bf16)
            if f % 2:
                cols = pl.ds((f - 1) * 128, 256)
                start_out(st.at[:, cols], hbm.at[:, cols], s)
        return finish

    def w_chunks(t, f):
        b = f % 2
        e = [("e", t, f)]

        def dgu():
            return _cat([_ld(dgu_s, (b, 0), 0, 256), _ld(dgu_s, (b, 1), 0, 256)])

        def add_halves(acc, v):
            for hf in range(2):
                part = v[:, hf * 128:(hf + 1) * 128]
                acc[t % 2, hf] = part if f == 0 else acc[t % 2, hf] + part

        def xf():
            lhs = _cat([_ld(wguL, (f, 0), 0, D), _ld(wguL, (f, 1), 0, D)])
            v = _nt(lhs, dgu())
            add_halves(xfT, v)
            return v

        def wgu_c():
            res = _nn(pair(xbTs, t, 0, D), dgu())
            accumulate(t, awg, f, res[:, 0:128],
                       dw_finish(dwg_st, dwg_h, SEM_DWG, f))
            accumulate(t, awu, f, res[:, 128:256],
                       dw_finish(dwu_st, dwu_h, SEM_DWU, f))
            return res

        def bt():
            v = _nt(_ld(wdL, (f,), 0, D), _ld(h_s, (b,), 0, 256))
            add_halves(bT, v)
            return v

        def wd_c():
            res = _nn(pair(dbT, t, 0, D), _ld(h_s, (b,), 0, 256))
            accumulate(t, awd, f, res, dw_finish(dwd_st, dwd_h, SEM_DWD, f))
            return res

        return [
            Unit(448, xf, needs=e + [("wL", f)], gives=[("xf", t, f)]),
            Unit(448, wgu_c, needs=e + [("xbTs", 2 * t), ("xbTs", 2 * t + 1)]),
            Unit(224, bt, needs=e + [("wL", f)], gives=[("bt", t, f)]),
            Unit(224, wd_c, needs=e + [("dbT", 2 * t), ("dbT", 2 * t + 1)])]

    def fin_unit(L):
        t, hf = L // 2, L % 2

        def fn():
            g = gs[L, 0:1, :]
            cols = slice(hf * 128, (hf + 1) * 128)
            dgb = None
            for r0 in range(0, D, 64):
                rows = slice(r0, r0 + 64)
                bt_v = bT[t % 2, hf, rows, :]
                part = dy_raw[rows, L * 128:(L + 1) * 128].astype(f32) * bt_v
                dgb = part if dgb is None else dgb + part
                out_st[t, rows, cols] = (
                    gaT[hf, rows, :] + (1.0 - g) * bt_v).astype(bf16)
            dgb = jnp.sum(dgb, axis=0, keepdims=True)
            ds = (dga[L, 0:1, :] - dgb) * g * (1.0 - g)
            ri = lax.broadcasted_iota(jnp.int32, (QKVP - QKV, 128), 0)
            _st(dqkv, (L,), QKV, jnp.where(ri == 0, ds, 0.0).astype(bf16))
            if hf == 1:
                start_out(out_st.at[t], out_h.at[:, pl.ds(t * 256, 256)],
                          SEM_OUT)
        needs = [("bt", t, NF - 1), ("ga", L), ("dl", L)]
        if hf == 1:
            needs.append(("fin", L - 1))
        lazy.append(Unit(120, fn, needs=needs, gives=[("fin", L)]))

    for L in range(NL):
        fin_unit(L)

    def tail_chunks(t):
        La, Lb = 2 * t, 2 * t + 1

        def ga(L):
            def fn():
                lhs = _cat([_ld(woT, (kt,), 0, D) for kt in range(4)])
                res = _nn(lhs, _ld(oT, (L,), 0, DP))
                gaT[L % 2] = res
                return res
            return Unit(D, fn,
                        needs=[("o", L)] + [("woT", kt) for kt in range(4)],
                        gives=[("ga", L)])

        def wo_c():
            res = _nt(pair(oT, t, 0, D), pair(dyT, t, 0, DP))

            def finish(j):
                def fin(v):
                    if j < 3:
                        dwo_st[:, j * 128:(j + 1) * 128] = v.astype(bf16)
                    else:
                        dwo_st[:, 384:448] = v[:, 0:64].astype(bf16)
                        start_out(dwo_st, dwo_h, SEM_DWO)
                return fin
            for j in range(4):
                accumulate(t, awo, j, res[:, j * 128:(j + 1) * 128], finish(j))
            return res

        grads = [(n, L) for n in ("dq", "dk", "dv") for L in (La, Lb)]

        def wq_c(j0, j1):
            def fn():
                res = _nt(pair(xT, t, 0, D), pair(dqkv, t, j0 * 128, j1 * 128))

                def finish(j):
                    def fin(v):
                        dwq_st[:, j * 128:(j + 1) * 128] = v.astype(bf16)
                        if j == j1 - 1:
                            cols = pl.ds(j0 * 128, (j1 - j0) * 128)
                            start_out(dwq_st.at[:, cols], dwq_h.at[:, cols],
                                      SEM_DWQ)
                    return fin
                for j in range(j0, j1):
                    accumulate(t, awq, j,
                               res[:, (j - j0) * 128:(j - j0 + 1) * 128],
                               finish(j))
                return res
            return Unit(224 * (j1 - j0), fn, needs=grads)

        def wq_end():
            j = NQ - 1
            res = _nt(pair(xT, t, 0, D), pair(dqkv, t, j * 128, (j + 1) * 128))

            def finish(v):
                dwq_se[...] = v[:, 0:64].astype(bf16)
                start_out(dwq_se, dwq_h.at[:, pl.ds(1280, 64)], SEM_DWQ)
                row = v.T[64:65, :]
                dgw_st[...] = row.astype(bf16).reshape(D)
                start_out(dgw_st, dgw_h, SEM_DGW)
            accumulate(t, awq, j, res, finish)
            return res

        def dx_c(L):
            def fn():
                lhs = _cat([_ld(wqkv, (j,), 0, D) for j in range(NQ)])
                om = 1.0 - gs[L, 0:1, :]
                v = _nn(lhs, _ld(dqkv, (L,), 0, QKVP))
                dx_st[L] = (v + om * xfT[t % 2, L % 2]).astype(bf16)
                start_out(dx_st.at[L], dx_h.at[:, pl.ds(L * 128, 128)], SEM_DX)
                return v
            return Unit(NQ * D // 4, fn,
                        needs=grads + [("fin", L), ("xf", t, NF - 1)]
                        + [("wq", j) for j in range(NQ)])

        return ([ga(La), ga(Lb),
                 Unit(896, wo_c, needs=[("o", La), ("o", Lb)], groups=2)],
                [wq_c(j0, j0 + 2) for j0 in range(0, NQ - 1, 2)],
                [Unit(224, wq_end, needs=grads + [("fin", La), ("fin", Lb)]),
                 dx_c(La), dx_c(Lb)])

    chunks = [barrier([("wo", None), ("dy", 0)], start_rest)]
    for L in range(NL):
        if L in DY_CUTS[1:-1]:
            chunks.append(barrier([("dy", L)]))
        if L == NL - 3:
            chunks.append(barrier([("x", 0), ("gw", None)] + w_keys(0)))
        chunks.append(p_chunk(L))

    waits = {0: w_keys(1), 2: [("wq", None)] + w_keys(2), 5: w_keys(3),
             9: [("x", X_CUTS[1])]}
    es = []
    marks = {}
    for t in range(NT):
        if t == 0:
            extra = {6 + 2 * i: [qkv_chunk(i)] for i in range(4)}
        else:
            extra = {}
            if 2 * t + 2 < NL:
                extra = {2: [qkv_chunk(2 * t + 2)], 5: [qkv_chunk(2 * t + 3)]}
            for f, part in zip((8, 10, 12), tail_chunks(t - 1)):
                extra[f] = part
        for f in range(NF):
            chunks += g_chunks(t, f)
            es += e_units(t, f)
            if t == 0 and f in waits:
                chunks.append(barrier(waits[f]))
            if f > 0:
                chunks += w_chunks(t, f - 1)
            chunks += extra.get(f, [])
            marks[(t, f)] = sum(c.cost for c in chunks)
        chunks += w_chunks(t, NF - 1)
    t_end = sum(c.cost for c in chunks)
    chunks += sum(tail_chunks(NT - 1), [])

    a0 = marks[(0, 7)]
    a1 = a0 + int((t_end - a0) * ATT_END)
    emit(chunks,
         [Queue(es, 0, 0, 2), Queue(att, a0, a1),
          Queue(wq_prep, marks[(0, 2)], marks[(0, 4)])],
         lazy)

    assert not in_flight
    for src, dst, s in out_flight:
        cp(src, dst, s).wait()


@jax.jit
def pallas_gated_mix__sliding_local_dilated__swiglu_ffn__prompt_kernel(
    A_x: jax.Array,
    A_wqkv: jax.Array,
    A_wo: jax.Array,
    B_x: jax.Array,
    B_w_gate: jax.Array,
    B_w_up: jax.Array,
    B_w_down: jax.Array,
    gate_w: jax.Array,
    grad_out: jax.Array,
):
    del B_x
    V = pltpu.VMEM
    scratch = [
        V((D, QKV), bf16), V((D, D), bf16), V((D,), bf16),
        V((D, S), bf16), V((D, S), bf16),
        V((D, F), bf16), V((D, F), bf16), V((D, F), bf16),
        V((D, 128), f32),
        V((NL, DP // 2, 128), u32), V((NL, DP // 2, 128), u32),
        V((NF, 2, DP // 2, 128), u32), V((NF, DP // 2, 128), u32),
        V((NF, 2, D // 2, 128), u32), V((NF, D // 2, 128), u32),
        V((NQ, D // 2, 128), u32), V((4, QKVP // 2, 128), u32),
        V((4, D // 2, 128), u32), V((4, D // 2, 128), u32),
        V((NL + 2, QKV + 32, 128), f32),
        V((NL + 2, D + 32, 128), f32),
        V((NL, 8, 128), f32),
        V((W, H, 128), f32), V((W, H, 128), f32), V((W, H, 128), f32),
        V((NL + 2, W, H, 128), f32), V((NL + 2, W, H, 128), f32),
        V((NL, 8, 128), f32),
        V((D + 32, 128), f32), V((D + 32, 128), f32),
        V((D + 32, 128), f32), V((D + 32, 128), f32),
        V((NL, DP // 2, 128), u32), V((NL, QKVP // 2, 128), u32),
        V((NT, 4, 128, 128), u32), V((NT, 4, 128, 128), u32),
        V((NL, D // 2, 128), u32), V((NL, D // 2, 128), u32),
        V((2, 2, 256, 128), f32), V((2, 256, 128), f32),
        V((2, 128, 128), u32), V((2, 2, 128, 128), u32),
        V((2, 2, D, 128), f32), V((2, D, 128), f32),
        V((2, 2, D, 128), f32),
        V((NF, D, 128), f32), V((NF, D, 128), f32), V((NF, D, 128), f32),
        V((4, D, 128), f32), V((NQ, D, 128), f32),
        V((NT, D, 256), bf16), V((NL, D, 128), bf16),
        V((D, F), bf16), V((D, F), bf16), V((D, F), bf16),
        V((D, D), bf16),
        V((D, (NQ - 1) * 128), bf16), V((D, 64), bf16),
        V((D,), bf16),
        pltpu.SemaphoreType.DMA((NSEM,)),
    ]
    any_spec = pl.BlockSpec(memory_space=pl.ANY)
    sds = jax.ShapeDtypeStruct
    outs = pl.pallas_call(
        _kernel,
        out_shape=(sds((D, S), bf16), sds((D, S), bf16), sds((D, QKV), bf16),
                   sds((D, D), bf16), sds((D, F), bf16), sds((D, F), bf16),
                   sds((D, F), bf16), sds((D,), bf16)),
        in_specs=[any_spec] * 8,
        out_specs=(any_spec,) * 8,
        scratch_shapes=scratch,
        compiler_params=pltpu.CompilerParams(
            vmem_limit_bytes=120 * 1024 * 1024),
    )(A_x[0].T, A_wqkv, A_wo, B_w_gate, B_w_up, B_w_down.T, gate_w,
      grad_out[0].T)
    out_t, dx_t, dwq, dwo, dwg, dwu, dwd_t, dgw = outs
    return (out_t.T[None], dx_t.T[None], dwq, dwo, dwg, dwu, dwd_t.T, dgw)
```

```python
import functools

import jax
import jax.numpy as jnp
from jax import lax
from jax.experimental import pallas as pl
from jax.experimental.pallas import tpu as pltpu

S = 2048
D = 448
DP = 512
H = 16
DH = 28
W = 8
F = 1792
NF = F // 128
NL = S // 128
NT = NL // 2
QKV = 3 * D
NQ = 11
QKVP = NQ * 128
SCALE = float(DH) ** -0.5

f32 = jnp.float32
bf16 = jnp.bfloat16
u32 = jnp.uint32

NH = 8
D_STEPS = 4
E_ROWS = 16
ATT_END = 0.95
DY_CUTS = (0, 1, 3, 6, 11, NL)
W_CUTS = (0, 1, 3, 6, NF)
X_CUTS = (0, 2, NL)

SEM_OUT = 10
NSEM = SEM_OUT + 1

_nn = functools.partial(jnp.dot, preferred_element_type=f32)
_nt = functools.partial(lax.dot_general,
                        dimension_numbers=(((1,), (1,)), ((), ())),
                        preferred_element_type=f32)


def _cat(parts):
    return jnp.concatenate(parts, axis=1)


def _ld(ref, idx, r0, r1):
    return pltpu.bitcast(ref[idx + (pl.ds(r0 // 2, (r1 - r0) // 2),)], bf16)


def _st(ref, idx, r0, val):
    ref[idx + (pl.ds(r0 // 2, val.shape[0] // 2),)] = pltpu.bitcast(val, u32)


class Unit:
    def __init__(self, cost, fn, needs=(), gives=(), steps=0, groups=1):
        self.cost, self.fn = cost, fn
        self.steps = steps
        self.groups = groups
        self.needs, self.gives = set(needs), set(gives)


class Queue:
    def __init__(self, units, t0, t1, per_chunk=1 << 30):
        self.units, self.t0, self.t1 = list(units), t0, t1
        self.per_chunk = per_chunk
        self.total = sum(u.cost for u in self.units)
        self.spent = 0
        self.pos = 0

    def target(self, t):
        if self.t1 <= self.t0:
            return self.total if t >= self.t0 else 0
        frac = (t - self.t0) / (self.t1 - self.t0)
        return self.total * min(max(frac, 0.0), 1.0)


def emit(chunks, queues, lazy):
    done = set()
    last = [None, 1]
    rel = {}
    state = dict(j=0, m=1)
    provider = {g: u for u in lazy for g in u.gives}
    where = {g: (q, i) for q in queues for i, u in enumerate(q.units)
             for g in u.gives}

    def release():
        res, groups = last
        j, m = min(state["j"], state["m"] - 1), state["m"]
        state["j"] += 1
        rows = res.shape[0] // 8
        per = res.shape[1] // 128 // groups
        pos = rows * groups * j // m
        r, c = (pos % rows) * 8, (pos // rows) * per * 128
        if (r, c) not in rel:
            rel[(r, c)] = jnp.minimum(jnp.abs(res[r:r + 8, c:c + 128]), 0.0)
        return rel[(r, c)]

    def run(u):
        for n in sorted(u.needs - done, key=str):
            force(n)
        if u.steps:
            u.fn(release)
        else:
            u.fn()
        done.update(u.gives)

    def step_queue(q):
        u = q.units[q.pos]
        q.pos += 1
        q.spent += u.cost
        run(u)

    def force(tok):
        if tok in done:
            return
        if tok in provider:
            run(provider[tok])
            return
        q, i = where[tok]
        while q.pos <= i:
            step_queue(q)

    def ready(u, extra):
        return all(n in done or n in extra
                   or (n in provider and ready(provider[n], extra))
                   for n in u.needs)

    t = 0
    for c in chunks:
        for n in sorted(c.needs - done, key=str):
            force(n)
        res = c.fn()
        if c.cost > 0:
            last[:] = [res, c.groups]
            rel.clear()
        done.update(c.gives)
        t += c.cost
        batch = []
        for q in queues:
            pos, spent, extra, n = q.pos, q.spent, set(), 0
            while (pos < len(q.units) and spent < q.target(t)
                   and n < q.per_chunk and ready(q.units[pos], extra)):
                u = q.units[pos]
                batch.append((q, u))
                extra |= u.gives
                spent += u.cost
                pos += 1
                n += 1
        state["j"] = 0
        state["m"] = max(sum(u.steps for _, u in batch), 1)
        for q, u in batch:
            if q.pos < len(q.units) and q.units[q.pos] is u:
                step_queue(q)
    assert all(q.pos == len(q.units) for q in queues)


def _kernel(xT_h, wq_h, wo_h, wg_h, wu_h, wd_h, gw_h, dyT_h,
            out_h, dx_h, dwq_h, dwo_h, dwg_h, dwu_h, dwd_h, dgw_h,
            wq_raw, wo_raw, gw_raw, x_raw, dy_raw, wg_raw, wu_raw, wd_raw,
            gwb, xT, dyT, wgu, wd, wguL, wdL, wqkv, wqkvT, wo, woT,
            qkv, pp, gs, lg, da, pr, at, dl, dga,
            o_st, dq_st, dk_st, dv_st, oT, dqkv,
            xb, dy, xbTs, dbT, gu_s, q_s, h_s, dgu_s,
            bT, gaT, xfT, awg, awu, awd, awo, awq,
            out_st, dx_st, dwg_st, dwu_st, dwd_st, dwo_st,
            dwq_st, dwq_se, dgw_st,
            sem):

    def cp(src, dst, s):
        return pltpu.make_async_copy(src, dst, sem.at[s])

    in_flight = {}

    def start_in(group, name, src, dst, t0=None, t1=None):
        if t0 is not None:
            cols = pl.ds(t0 * 128, (t1 - t0) * 128)
            src, dst = src.at[:, cols], dst.at[:, cols]
        in_flight.setdefault(group, []).append(((name, t0), (src, dst, group)))
        cp(src, dst, group).start()

    def pieces(key):
        name, t0 = key
        if t0 is None:
            return [name]
        cuts = dict(dy=DY_CUTS, x=X_CUTS).get(name, W_CUTS)
        return [(name, i) for i in range(t0, cuts[cuts.index(t0) + 1])]

    def barrier(group, keys, then=None):
        def fn():
            copies = in_flight.pop(group)
            assert sorted(k for k, _ in copies) == sorted(keys)
            for _, args in copies:
                cp(*args).wait()
            if then is not None:
                then()
        return Unit(0, fn, gives=[("dma", g) for k in keys for g in pieces(k)])

    out_flight = []

    def start_out(src, dst):
        out_flight.append((src, dst, SEM_OUT))
        cp(src, dst, SEM_OUT).start()

    def start_w(group, i):
        for nm, h_, r_ in (("wg", wg_h, wg_raw), ("wu", wu_h, wu_raw),
                           ("wd", wd_h, wd_raw)):
            start_in(group, nm, h_, r_, W_CUTS[i], W_CUTS[i + 1])

    def w_keys(i):
        return [(nm, W_CUTS[i]) for nm in ("wg", "wu", "wd")]

    dy_groups = list(zip(DY_CUTS[:-1], DY_CUTS[1:]))
    start_in(0, "wo", wo_h, wo_raw)
    for i in range(2):
        start_in(i, "dy", dyT_h, dy_raw, *dy_groups[i])

    def start_rest():
        for i in range(2, 5):
            start_in(i, "dy", dyT_h, dy_raw, *dy_groups[i])
        start_in(5, "x", xT_h, x_raw, X_CUTS[0], X_CUTS[1])
        start_in(5, "gw", gw_h, gw_raw)
        start_w(5, 0)
        start_w(6, 1)
        start_in(7, "wq", wq_h, wq_raw)
        start_w(7, 2)
        start_w(8, 3)
        start_in(9, "x", xT_h, x_raw, X_CUTS[1], X_CUTS[2])

    lane16 = lax.broadcasted_iota(jnp.int32, (H, 128), 1)
    lane8 = lax.broadcasted_iota(jnp.int32, (NH, 128), 1)

    def zeros(shape, dt):
        return jnp.zeros(shape, dt)

    def col(raw, i):
        return raw[:, i * 128:(i + 1) * 128]

    lazy = []

    def padded(tile):
        return jnp.concatenate([tile, zeros((DP - D, 128), bf16)], axis=0)

    def repack_unit(name, raw, i, dst):
        def fn():
            dst[i] = pltpu.bitcast(padded(col(raw, i)), u32)
        lazy.append(Unit(30, fn, needs=[("dma", (name, i))],
                         gives=[(name + "T", i)]))

    for L in range(NL):
        repack_unit("dy", dy_raw, L, dyT)
        repack_unit("x", x_raw, L, xT)

    def w_units(f):
        needs = [("dma", (n, f)) for n in ("wg", "wu", "wd")]

        def as_rhs():
            g, u, d_ = col(wg_raw, f), col(wu_raw, f), col(wd_raw, f)
            wgu[f, 0] = pltpu.bitcast(padded(g), u32)
            wgu[f, 1] = pltpu.bitcast(padded(u), u32)
            wd[f] = pltpu.bitcast(padded(d_), u32)
        lazy.append(Unit(60, as_rhs, needs=needs, gives=[("w", f)]))

        def as_lhs():
            wguL[f, 0] = pltpu.bitcast(col(wg_raw, f), u32)
            wguL[f, 1] = pltpu.bitcast(col(wu_raw, f), u32)
            wdL[f] = pltpu.bitcast(col(wd_raw, f), u32)
        lazy.append(Unit(60, as_lhs, needs=needs, gives=[("wL", f)]))

    for f in range(NF):
        w_units(f)

    def end_tile(raw, c0):
        return _cat([raw[:, c0:c0 + 64], zeros((D, 64), bf16)])

    def prep_wo():
        for k in range(3):
            wo[k] = pltpu.bitcast(col(wo_raw, k), u32)
        wo[3] = pltpu.bitcast(end_tile(wo_raw, 384), u32)
    lazy.append(Unit(60, prep_wo, needs=[("dma", "wo")], gives=["wo"]))

    def wot_unit(kt):
        def fn():
            r0 = kt * 128
            r1 = min(r0 + 128, D)
            blk = _cat([_ld(wo, (k,), r0, r1) for k in range(4)])
            if r1 - r0 < 128:
                blk = jnp.concatenate(
                    [blk, zeros((128 - (r1 - r0), DP), bf16)], axis=0)
            _st(woT, (kt,), 0, blk.T[0:D, :])
        lazy.append(Unit(150, fn, needs=["wo"], gives=[("woT", kt)]))

    for kt in range(4):
        wot_unit(kt)

    def gwb_unit():
        row = gw_raw[...].reshape(1, D).astype(f32)
        gwb[...] = jnp.broadcast_to(row, (128, D)).T
    lazy.append(Unit(150, gwb_unit, needs=[("dma", "gw")], gives=["gwb"]))

    def wq_unit(j):
        def fn():
            if j < NQ - 1:
                tile = col(wq_raw, j)
            else:
                li = lax.broadcasted_iota(jnp.int32, (D, 128), 1)
                tile = jnp.where(li == 64, gwb[...],
                                 end_tile(wq_raw, 1280).astype(f32)).astype(bf16)
            wqkv[j] = pltpu.bitcast(tile, u32)
            tile = padded(tile)
            for kt in range(4):
                _st(wqkvT, (kt,), j * 128, tile[kt * 128:(kt + 1) * 128, :].T)
        needs = [("dma", "wq")] + (["gwb"] if j == NQ - 1 else [])
        return Unit(250, fn, needs=needs, gives=[("wq", j)])

    wq_prep = [wq_unit(j) for j in range(NQ)]

    def gate_unit(L):
        def fn():
            z = jnp.sum(col(x_raw, L).astype(f32) * gwb[...], axis=0,
                        keepdims=True)
            gs[L] = jnp.broadcast_to(jax.nn.sigmoid(z), (8, 128))
        lazy.append(Unit(60, fn, needs=[("dma", ("x", L)), "gwb"],
                         gives=[("g", L)]))

    def tr_unit(L, src, stag, dst, tag):
        def fn():
            for kt in range(4):
                _st(dst, (L // 2, kt), (L % 2) * 128,
                    _ld(src, (L,), kt * 128, (kt + 1) * 128).T)
        lazy.append(Unit(220, fn, needs=[(stag, L)], gives=[(tag, L)]))

    def scale_unit(L, raw, key, dst, tag):
        def fn():
            om = 1.0 - gs[L, 0:1, :]
            _st(dst, (L,), 0, (col(raw, L).astype(f32) * om).astype(bf16))
        lazy.append(Unit(60, fn, needs=[("dma", (key, L)), ("g", L)],
                         gives=[(tag, L)]))

    for L in range(NL):
        gate_unit(L)
        tr_unit(L, dyT, "dyT", dy, "dy")
        tr_unit(L, xT, "xT", xb, "xb")
        scale_unit(L, dy_raw, "dy", dbT, "dbT")
        scale_unit(L, x_raw, "x", xbTs, "xbTs")

    def zero_unit(tag, ref, idx, shape, dt):
        def fn():
            ref[idx] = zeros(shape, dt)
        lazy.append(Unit(10, fn, gives=[tag]))

    zero_unit("kv_halo", qkv, (0, pl.ds(D, 2 * D)), (2 * D, 128), f32)
    zero_unit("q_halo", qkv, (NL + 1, pl.ds(0, D)), (D, 128), f32)
    zero_unit("p_halo", pp, (NL + 1, pl.ds(0, D)), (D, 128), f32)
    zero_unit("at_halo", at, (NL + 1,), (W, H, 128), f32)
    zero_unit("dl_halo", dl, (NL + 1,), (W, H, 128), f32)
    for L in range(NL):
        zero_unit(("oz", L), oT, (L, pl.ds(D // 2, DP // 2 - D // 2)),
                  (DP // 2 - D // 2, 128), u32)

    def heads(ref, i, off, d, h0):
        return ref[i, pl.ds(off + h0 * DH + d, NH, stride=DH), :]

    from_prev = {w: lane8 >= 128 - 2 * w for w in range(1, W)}
    from_next = {w: lane8 < 2 * w for w in range(1, W)}

    def shift_r(cur, prev, w):
        return pltpu.roll(lax.select(from_prev[w], prev, cur), 2 * w, 1)

    def shift_l(cur, nxt, w):
        return pltpu.roll(lax.select(from_next[w], nxt, cur), 128 - 2 * w, 1)

    def head_groups(build, needs, gives):
        units = []
        for h0 in range(0, H, NH):
            fn_of = build(h0)
            for d0 in range(0, DH, D_STEPS):
                d1 = min(d0 + D_STEPS, DH)
                units.append(Unit((W - 1) * 8 * (d1 - d0) // 3 + 4,
                                  fn_of(d0, d1), steps=d1 - d0))
        units[0].needs |= set(needs)
        units[-1].gives |= set(gives)
        return units

    def logit_units(L):
        li = L + 1

        def build(h0):
            acc = [None] * W

            def make(d0, d1):
                def fn(rel):
                    for d in range(d0, d1):
                        a = heads(qkv, li, 0, d, h0)
                        bc = heads(qkv, li, D, d, h0) + rel()
                        bp = heads(qkv, li - 1, D, d, h0)
                        for w in range(W):
                            t = a * (shift_r(bc, bp, w) if w else bc)
                            acc[w] = t if acc[w] is None else acc[w] + t
                    if d1 == DH:
                        for w in range(W):
                            lg[w, h0:h0 + NH, :] = acc[w]
                return fn
            return make

        needs = [("qkv", L)] + ([("qkv", L - 1)] if L else ["kv_halo"])
        return head_groups(build, needs, [("lg", L)])

    def softmax_unit(L):
        li = L + 1

        def fn():
            g = gs[L, 0:1, :]
            lo = [lg[w] * SCALE for w in range(W)]
            if L == 0:
                lo = [lo[0]] + [jnp.where(lane16 >= 2 * w, lo[w], -1e9)
                                for w in range(1, W)]
            m = lo[0]
            for w in range(1, W):
                m = jnp.maximum(m, lo[w])
            e = [jnp.exp(lo[w] - m) for w in range(W)]
            s = e[0]
            for w in range(1, W):
                s = s + e[w]
            r = 1.0 / s
            for w in range(W):
                p = e[w] * r
                pr[w] = p
                at[li, w] = p * g
        return Unit(40, fn, needs=[("lg", L), ("g", L)], gives=[("p", L)])

    def value_units(L):
        li = L + 1

        def build(h0):
            acc = [None] * W
            coef = [None] * W

            def make(d0, d1):
                def fn(rel):
                    if d0 == 0:
                        for w in range(W):
                            coef[w] = at[li, w, h0:h0 + NH, :]
                    for d in range(d0, d1):
                        a = heads(pp, li, 0, d, h0)
                        bc = heads(qkv, li, 2 * D, d, h0) + rel()
                        bp = heads(qkv, li - 1, 2 * D, d, h0)
                        r = None
                        for w in range(W):
                            bs = shift_r(bc, bp, w) if w else bc
                            t = a * bs
                            acc[w] = t if acc[w] is None else acc[w] + t
                            t = coef[w] * bs
                            r = t if r is None else r + t
                        o_st[pl.ds(h0 * DH + d, NH, stride=DH), :] = r
                    if d1 == DH:
                        for w in range(W):
                            da[w, h0:h0 + NH, :] = acc[w]
                return fn
            return make

        return head_groups(build, [("p", L), ("P", L)], [("v", L)])

    def softmax_bwd_unit(L):
        li = L + 1

        def fn():
            gsc = gs[L, 0:1, :] * SCALE
            p = [pr[w] for w in range(W)]
            dd = [da[w] for w in range(W)]
            dot = p[0] * dd[0]
            for w in range(1, W):
                dot = dot + p[w] * dd[w]
            dga[L] = jnp.broadcast_to(
                jnp.sum(dot, axis=0, keepdims=True), (8, 128))
            for w in range(W):
                dl[li, w] = p[w] * (dd[w] - dot) * gsc
        return Unit(30, fn, needs=[("v", L)], gives=[("dl", L)])

    def combine_units(tag, needs, load_coef, load_pair, shift, dst):
        def build(h0):
            coef = [None] * W

            def make(d0, d1):
                def fn(rel):
                    if d0 == 0:
                        for w in range(W):
                            coef[w] = load_coef(h0, w)
                    for d in range(d0, d1):
                        cur, other = load_pair(d, h0)
                        cur = cur + rel()
                        r = coef[0] * cur
                        for w in range(1, W):
                            r = r + coef[w] * shift(cur, other, w)
                        dst[pl.ds(h0 * DH + d, NH, stride=DH), :] = r
                return fn
            return make

        return head_groups(build, needs, [tag])

    def dq_units(L):
        li = L + 1
        return combine_units(
            ("dqs", L), [("dl", L)],
            lambda h0, w: dl[li, w, h0:h0 + NH, :],
            lambda d, h0: (heads(qkv, li, D, d, h0),
                           heads(qkv, li - 1, D, d, h0)),
            shift_r, dq_st)

    def scatter_units(tag, needs, L, coef_ref, a_ref, dst):
        li = L + 1

        def load_coef(h0, w):
            cur = coef_ref[li, w, h0:h0 + NH, :]
            if w == 0:
                return cur
            return shift_l(cur, coef_ref[li + 1, w, h0:h0 + NH, :], w)
        return combine_units(
            tag, needs, load_coef,
            lambda d, h0: (heads(a_ref, li, 0, d, h0),
                           heads(a_ref, li + 1, 0, d, h0)),
            shift_l, dst)

    def pack_unit(tag, needs, src, dst, L, r0):
        def fn():
            _st(dst, (L,), r0, src[0:D, :].astype(bf16))
        return Unit(20, fn, needs=needs, gives=[tag])

    def fwd_attn(L):
        u = logit_units(L)
        u.append(softmax_unit(L))
        u += value_units(L)
        u.append(pack_unit(("o", L), [("v", L), ("oz", L)], o_st, oT, L, 0))
        u.append(softmax_bwd_unit(L))
        u += dq_units(L)
        u.append(pack_unit(("dq", L), [("dqs", L)], dq_st, dqkv, L, 0))
        return u

    def bwd_attn(L):
        if L + 1 < NL:
            nk = [("dl", L + 1), ("qkv", L + 1)]
            nv = [("dl", L + 1), ("P", L + 1)]
        else:
            nk = ["dl_halo", "q_halo"]
            nv = ["at_halo", "p_halo"]
        u = scatter_units(("dks", L), [("dl", L)] + nk, L, dl, qkv, dk_st)
        u.append(pack_unit(("dk", L), [("dks", L)], dk_st, dqkv, L, D))
        u += scatter_units(("dvs", L), [("dl", L)] + nv, L, at, pp, dv_st)
        u.append(pack_unit(("dv", L), [("dvs", L)], dv_st, dqkv, L, 2 * D))
        return u

    att = fwd_attn(0)
    for L in range(1, NL):
        att += fwd_attn(L)
        att += bwd_attn(L - 1)
    att += bwd_attn(NL - 1)

    def p_chunk(L):
        def fn():
            lhs = _cat([_ld(wo, (k,), 0, D) for k in range(4)])
            res = _nn(lhs, _ld(dyT, (L,), 0, DP))
            pp[L + 1, 0:D, :] = res
            return res
        return Unit(D, fn, needs=["wo", ("dyT", L)], gives=[("P", L)])

    def qkv_chunk(L):
        def fn():
            lhs = _cat([_ld(wqkvT, (kt,), 0, QKV) for kt in range(4)])
            res = _nn(lhs, _ld(xT, (L,), 0, DP))
            qkv[L + 1, 0:QKV, :] = res
            return res
        return Unit(QKV, fn,
                    needs=[("xT", L)] + [("wq", j) for j in range(NQ)],
                    gives=[("qkv", L)])

    def pair(ref, t, r0, r1):
        return _cat([_ld(ref, (2 * t,), r0, r1), _ld(ref, (2 * t + 1,), r0, r1)])

    def nat(ref, t):
        return _cat([_ld(ref, (t, kt), 0, 256) for kt in range(4)])

    def g_chunks(t, f):
        b = f % 2

        def gu():
            rhs = _cat([_ld(wgu, (f, 0), 0, DP), _ld(wgu, (f, 1), 0, DP)])
            res = _nn(nat(xb, t), rhs)
            gu_s[b, 0] = res[:, 0:128]
            gu_s[b, 1] = res[:, 128:256]
            return res

        def q():
            res = _nn(nat(dy, t), _ld(wd, (f,), 0, DP))
            q_s[b] = res
            return res
        return [Unit(512, gu, needs=[("xb", 2 * t), ("xb", 2 * t + 1), ("w", f)],
                     gives=[("gu", t, f)]),
                Unit(256, q, needs=[("dy", 2 * t), ("dy", 2 * t + 1), ("w", f)],
                     gives=[("q", t, f)])]

    def e_units(t, f):
        b = f % 2

        def mk(r0):
            def fn():
                r1 = r0 + E_ROWS
                z = gu_s[b, 0, r0:r1, :]
                u = gu_s[b, 1, r0:r1, :]
                q = q_s[b, r0:r1, :]
                sg = 0.5 * jnp.tanh(0.5 * z) + 0.5
                si = z * sg
                _st(h_s, (b,), r0, (si * u).astype(bf16))
                dsi = sg + si * (1.0 - sg)
                _st(dgu_s, (b, 0), r0, (q * u * dsi).astype(bf16))
                _st(dgu_s, (b, 1), r0, (q * si).astype(bf16))
            return fn
        return [Unit(E_ROWS // 2, mk(r0), needs=[("gu", t, f), ("q", t, f)],
                     gives=[("e", t, f)] if r0 + E_ROWS == 256 else [])
                for r0 in range(0, 256, E_ROWS)]

    def accumulate(t, acc, idx, val, finish):
        v = val if t == 0 else acc[idx] + val
        if t == NT - 1:
            finish(v)
        else:
            acc[idx] = v

    def dw_finish(st, hbm, f):
        def finish(v):
            st[:, f * 128:(f + 1) * 128] = v.astype(bf16)
            if f % 2:
                cols = pl.ds((f - 1) * 128, 256)
                start_out(st.at[:, cols], hbm.at[:, cols])
        return finish

    def w_chunks(t, f):
        b = f % 2
        e = [("e", t, f)]

        def dgu():
            return _cat([_ld(dgu_s, (b, 0), 0, 256), _ld(dgu_s, (b, 1), 0, 256)])

        def add_halves(acc, v):
            for hf in range(2):
                part = v[:, hf * 128:(hf + 1) * 128]
                acc[t % 2, hf] = part if f == 0 else acc[t % 2, hf] + part

        def xf():
            lhs = _cat([_ld(wguL, (f, 0), 0, D), _ld(wguL, (f, 1), 0, D)])
            v = _nt(lhs, dgu())
            add_halves(xfT, v)
            return v

        def wgu_c():
            res = _nn(pair(xbTs, t, 0, D), dgu())
            accumulate(t, awg, f, res[:, 0:128],
                       dw_finish(dwg_st, dwg_h, f))
            accumulate(t, awu, f, res[:, 128:256],
                       dw_finish(dwu_st, dwu_h, f))
            return res

        def bt():
            v = _nt(_ld(wdL, (f,), 0, D), _ld(h_s, (b,), 0, 256))
            add_halves(bT, v)
            return v

        def wd_c():
            res = _nn(pair(dbT, t, 0, D), _ld(h_s, (b,), 0, 256))
            accumulate(t, awd, f, res, dw_finish(dwd_st, dwd_h, f))
            return res

        return [
            Unit(448, xf, needs=e + [("wL", f)], gives=[("xf", t, f)]),
            Unit(448, wgu_c, needs=e + [("xbTs", 2 * t), ("xbTs", 2 * t + 1)]),
            Unit(224, bt, needs=e + [("wL", f)], gives=[("bt", t, f)]),
            Unit(224, wd_c, needs=e + [("dbT", 2 * t), ("dbT", 2 * t + 1)])]

    def fin_unit(L):
        t, hf = L // 2, L % 2

        def fn():
            g = gs[L, 0:1, :]
            cols = slice(hf * 128, (hf + 1) * 128)
            dgb = None
            for r0 in range(0, D, 64):
                rows = slice(r0, r0 + 64)
                bt_v = bT[t % 2, hf, rows, :]
                part = dy_raw[rows, L * 128:(L + 1) * 128].astype(f32) * bt_v
                dgb = part if dgb is None else dgb + part
                out_st[t, rows, cols] = (
                    gaT[hf, rows, :] + (1.0 - g) * bt_v).astype(bf16)
            dgb = jnp.sum(dgb, axis=0, keepdims=True)
            ds = (dga[L, 0:1, :] - dgb) * g * (1.0 - g)
            ri = lax.broadcasted_iota(jnp.int32, (QKVP - QKV, 128), 0)
            _st(dqkv, (L,), QKV, jnp.where(ri == 0, ds, 0.0).astype(bf16))
            if hf == 1:
                start_out(out_st.at[t], out_h.at[:, pl.ds(t * 256, 256)])
        needs = [("bt", t, NF - 1), ("ga", L), ("dl", L)]
        if hf == 1:
            needs.append(("fin", L - 1))
        lazy.append(Unit(120, fn, needs=needs, gives=[("fin", L)]))

    for L in range(NL):
        fin_unit(L)

    def tail_chunks(t):
        La, Lb = 2 * t, 2 * t + 1

        def ga(L):
            def fn():
                lhs = _cat([_ld(woT, (kt,), 0, D) for kt in range(4)])
                res = _nn(lhs, _ld(oT, (L,), 0, DP))
                gaT[L % 2] = res
                return res
            return Unit(D, fn,
                        needs=[("o", L)] + [("woT", kt) for kt in range(4)],
                        gives=[("ga", L)])

        def wo_c():
            res = _nt(pair(oT, t, 0, D), pair(dyT, t, 0, DP))

            def finish(j):
                def fin(v):
                    if j < 3:
                        dwo_st[:, j * 128:(j + 1) * 128] = v.astype(bf16)
                    else:
                        dwo_st[:, 384:448] = v[:, 0:64].astype(bf16)
                        start_out(dwo_st, dwo_h)
                return fin
            for j in range(4):
                accumulate(t, awo, j, res[:, j * 128:(j + 1) * 128], finish(j))
            return res

        grads = [(n, L) for n in ("dq", "dk", "dv") for L in (La, Lb)]

        def wq_c(j0, j1):
            def fn():
                res = _nt(pair(xT, t, 0, D), pair(dqkv, t, j0 * 128, j1 * 128))

                def finish(j):
                    def fin(v):
                        dwq_st[:, j * 128:(j + 1) * 128] = v.astype(bf16)
                        if j == j1 - 1:
                            cols = pl.ds(j0 * 128, (j1 - j0) * 128)
                            start_out(dwq_st.at[:, cols], dwq_h.at[:, cols])
                    return fin
                for j in range(j0, j1):
                    accumulate(t, awq, j,
                               res[:, (j - j0) * 128:(j - j0 + 1) * 128],
                               finish(j))
                return res
            return Unit(224 * (j1 - j0), fn, needs=grads)

        def wq_end():
            j = NQ - 1
            res = _nt(pair(xT, t, 0, D), pair(dqkv, t, j * 128, (j + 1) * 128))

            def finish(v):
                dwq_se[...] = v[:, 0:64].astype(bf16)
                start_out(dwq_se, dwq_h.at[:, pl.ds(1280, 64)])
                row = v.T[64:65, :]
                dgw_st[...] = row.astype(bf16).reshape(D)
                start_out(dgw_st, dgw_h)
            accumulate(t, awq, j, res, finish)
            return res

        def dx_c(L):
            def fn():
                lhs = _cat([_ld(wqkv, (j,), 0, D) for j in range(NQ)])
                om = 1.0 - gs[L, 0:1, :]
                v = _nn(lhs, _ld(dqkv, (L,), 0, QKVP))
                dx_st[L] = (v + om * xfT[t % 2, L % 2]).astype(bf16)
                start_out(dx_st.at[L], dx_h.at[:, pl.ds(L * 128, 128)])
                return v
            return Unit(NQ * D // 4, fn,
                        needs=grads + [("fin", L), ("xf", t, NF - 1)]
                        + [("wq", j) for j in range(NQ)])

        return ([ga(La), ga(Lb),
                 Unit(896, wo_c, needs=[("o", La), ("o", Lb)], groups=2)],
                [wq_c(j0, j0 + 2) for j0 in range(0, NQ - 1, 2)],
                [Unit(224, wq_end, needs=grads + [("fin", La), ("fin", Lb)]),
                 dx_c(La), dx_c(Lb)])

    chunks = [barrier(0, [("wo", None), ("dy", 0)], start_rest)]
    for L in range(NL):
        if L in DY_CUTS[1:-1]:
            chunks.append(barrier(DY_CUTS.index(L), [("dy", L)]))
        if L == NL - 3:
            chunks.append(barrier(5, [("x", 0), ("gw", None)] + w_keys(0)))
        chunks.append(p_chunk(L))

    waits = {0: (6, w_keys(1)), 2: (7, [("wq", None)] + w_keys(2)),
             5: (8, w_keys(3)), 9: (9, [("x", X_CUTS[1])])}
    es = []
    marks = {}
    for t in range(NT):
        if t == 0:
            extra = {6 + 2 * i: [qkv_chunk(i)] for i in range(4)}
        else:
            extra = {}
            if 2 * t + 2 < NL:
                extra = {2: [qkv_chunk(2 * t + 2)], 5: [qkv_chunk(2 * t + 3)]}
            for f, part in zip((8, 10, 12), tail_chunks(t - 1)):
                extra[f] = part
        for f in range(NF):
            chunks += g_chunks(t, f)
            es += e_units(t, f)
            if t == 0 and f in waits:
                chunks.append(barrier(*waits[f]))
            if f > 0:
                chunks += w_chunks(t, f - 1)
            chunks += extra.get(f, [])
            marks[(t, f)] = sum(c.cost for c in chunks)
        chunks += w_chunks(t, NF - 1)
    t_end = sum(c.cost for c in chunks)
    chunks += sum(tail_chunks(NT - 1), [])

    a0 = marks[(0, 7)]
    a1 = a0 + int((t_end - a0) * ATT_END)
    emit(chunks,
         [Queue(es, 0, 0, 2), Queue(att, a0, a1),
          Queue(wq_prep, marks[(0, 2)], marks[(0, 4)])],
         lazy)

    assert not in_flight
    for src, dst, s in out_flight:
        cp(src, dst, s).wait()


@jax.jit
def pallas_gated_mix__sliding_local_dilated__swiglu_ffn__prompt_kernel(
    A_x: jax.Array,
    A_wqkv: jax.Array,
    A_wo: jax.Array,
    B_x: jax.Array,
    B_w_gate: jax.Array,
    B_w_up: jax.Array,
    B_w_down: jax.Array,
    gate_w: jax.Array,
    grad_out: jax.Array,
):
    del B_x
    V = pltpu.VMEM
    scratch = [
        V((D, QKV), bf16), V((D, D), bf16), V((D,), bf16),
        V((D, S), bf16), V((D, S), bf16),
        V((D, F), bf16), V((D, F), bf16), V((D, F), bf16),
        V((D, 128), f32),
        V((NL, DP // 2, 128), u32), V((NL, DP // 2, 128), u32),
        V((NF, 2, DP // 2, 128), u32), V((NF, DP // 2, 128), u32),
        V((NF, 2, D // 2, 128), u32), V((NF, D // 2, 128), u32),
        V((NQ, D // 2, 128), u32), V((4, QKVP // 2, 128), u32),
        V((4, D // 2, 128), u32), V((4, D // 2, 128), u32),
        V((NL + 2, QKV + 32, 128), f32),
        V((NL + 2, D + 32, 128), f32),
        V((NL, 8, 128), f32),
        V((W, H, 128), f32), V((W, H, 128), f32), V((W, H, 128), f32),
        V((NL + 2, W, H, 128), f32), V((NL + 2, W, H, 128), f32),
        V((NL, 8, 128), f32),
        V((D + 32, 128), f32), V((D + 32, 128), f32),
        V((D + 32, 128), f32), V((D + 32, 128), f32),
        V((NL, DP // 2, 128), u32), V((NL, QKVP // 2, 128), u32),
        V((NT, 4, 128, 128), u32), V((NT, 4, 128, 128), u32),
        V((NL, D // 2, 128), u32), V((NL, D // 2, 128), u32),
        V((2, 2, 256, 128), f32), V((2, 256, 128), f32),
        V((2, 128, 128), u32), V((2, 2, 128, 128), u32),
        V((2, 2, D, 128), f32), V((2, D, 128), f32),
        V((2, 2, D, 128), f32),
        V((NF, D, 128), f32), V((NF, D, 128), f32), V((NF, D, 128), f32),
        V((4, D, 128), f32), V((NQ, D, 128), f32),
        V((NT, D, 256), bf16), V((NL, D, 128), bf16),
        V((D, F), bf16), V((D, F), bf16), V((D, F), bf16),
        V((D, D), bf16),
        V((D, (NQ - 1) * 128), bf16), V((D, 64), bf16),
        V((D,), bf16),
        pltpu.SemaphoreType.DMA((NSEM,)),
    ]
    any_spec = pl.BlockSpec(memory_space=pl.ANY)
    sds = jax.ShapeDtypeStruct
    outs = pl.pallas_call(
        _kernel,
        out_shape=(sds((D, S), bf16), sds((D, S), bf16), sds((D, QKV), bf16),
                   sds((D, D), bf16), sds((D, F), bf16), sds((D, F), bf16),
                   sds((D, F), bf16), sds((D,), bf16)),
        in_specs=[any_spec] * 8,
        out_specs=(any_spec,) * 8,
        scratch_shapes=scratch,
        compiler_params=pltpu.CompilerParams(
            vmem_limit_bytes=120 * 1024 * 1024),
    )(A_x[0].T, A_wqkv, A_wo, B_w_gate, B_w_up, B_w_down.T, gate_w,
      grad_out[0].T)
    out_t, dx_t, dwq, dwo, dwg, dwu, dwd_t, dgw = outs
    return (out_t.T[None], dx_t.T[None], dwq, dwo, dwg, dwu, dwd_t.T, dgw)
```
